```python
import os as _os
_os.environ.setdefault("JAX_PLATFORMS", "cpu")
import jax
import jax.numpy as jnp

def _softmax(x, axis=-1):
    return jax.nn.softmax(x, axis=axis)
def _gelu(x):
    return jax.nn.gelu(x, approximate=True)
def _silu(x):
    return jax.nn.silu(x)
def _sigmoid(x):
    return jax.nn.sigmoid(x)
def _layernorm(x, axis=-1, eps=1e-5):
    m = jnp.mean(x, axis=axis, keepdims=True)
    v = jnp.var(x, axis=axis, keepdims=True)
    return (x - m) / jnp.sqrt(v + eps)
def _scatter_add(tgt, idx, src, axis=0):
    return tgt.at[idx].add(src)
def _segment_sum(src, seg, n):
    return jax.ops.segment_sum(src, seg, n)
class _Rng:
    def __init__(self, key):
        self._k = key
    def _next(self):
        self._k, sub = jax.random.split(self._k)
        return sub
    def normal(self, shape):
        return jax.random.normal(self._next(), shape, dtype=jnp.bfloat16)
    def randint(self, lo, hi, shape):
        return jax.random.randint(self._next(), shape, lo, hi, dtype=jnp.int32)
    def uniform(self, shape, lo=0.0, hi=1.0):
        return jax.random.uniform(self._next(), shape, jnp.bfloat16, lo, hi)
    def permutation(self, n):
        return jax.random.permutation(self._next(), n)


kernel_name = 'concat_heads__gqa_block_cached__mha_block_cached__near_ridge'

def setup_inputs():
    _rng = _Rng(jax.random.key(int.from_bytes(__import__("os").urandom(4), "little")))
    _w = (lambda a: (lambda t: t.astype(jnp.bfloat16) if jnp.issubdtype(t.dtype, jnp.floating) else t)(jnp.asarray(a)))
    def _A_setup():
        B, Sq, D = 16, 32, 1024
        Hq, Hkv, Sk, Dh = 32, 4, 32, 128
        assert Hq % Hkv == 0, (Hq, Hkv)
        return {
            "x": _w((lambda *s: _rng.normal(s) * 0.8)(B, Sq, D)),
            "k_cache": _w((lambda *s: _rng.normal(s) * 0.8)(B, Hkv, Sk, Dh)),
            "v_cache": _w((lambda *s: _rng.normal(s) * 0.05)(B, Hkv, Sk, Dh)),
            "wq": _w((lambda *s: _rng.normal(s) * 0.8)(D, Hq * Dh) * (D ** -0.5)),
            "wo": _w((lambda *s: _rng.normal(s) * 0.05)(Hq * Dh, D) * ((Hq * Dh) ** -0.5)),
        }
    _A_in = _A_setup()

    def _B_setup():
        B, Sq, D = 16, 32, 1024
        H, Sk, Dh = 32, 32, 128
        return {
            "x": _w((lambda *s: _rng.normal(s) * 0.8)(B, Sq, D)),
            "k_cache": _w((lambda *s: _rng.normal(s) * 0.8)(B, H, Sk, Dh)),
            "v_cache": _w((lambda *s: _rng.normal(s) * 0.05)(B, H, Sk, Dh)),
            "wq": _w((lambda *s: _rng.normal(s) * 0.8)(D, H * Dh) * (D ** -0.5)),
            "wo": _w((lambda *s: _rng.normal(s) * 0.05)(H * Dh, D) * ((H * Dh) ** -0.5)),
        }
    _B_in = _B_setup()

    return {
        "A_x": _A_in["x"],
        "A_k_cache": _A_in["k_cache"],
        "A_v_cache": _A_in["v_cache"],
        "A_wq": _A_in["wq"],
        "A_wo": _A_in["wo"],
        "B_x": _B_in["x"],
        "B_k_cache": _B_in["k_cache"],
        "B_v_cache": _B_in["v_cache"],
        "B_wq": _B_in["wq"],
        "B_wo": _B_in["wo"],
    }

def reference(A_x, A_k_cache, A_v_cache, A_wq, A_wo, B_x, B_k_cache, B_v_cache, B_wq, B_wo):
    def _A_ref(x, k_cache, v_cache, wq, wo):
        B, Sq, D = x.shape
        Hq, Dh = 32, 128
        Hkv = k_cache.shape[1]
        rep = Hq // Hkv
        q = (lambda x, *d: x.transpose(*d))((x @ wq).reshape(B, Sq, Hq, Dh), 0, 2, 1, 3)
        k = jnp.repeat(k_cache, rep, axis=1)
        v = jnp.repeat(v_cache, rep, axis=1)
        scores = jnp.einsum("bhqd,bhkd->bhqk", q, k) * (Dh ** -0.5)
        p = _softmax(scores, axis=-1)
        o = jnp.einsum("bhqk,bhkd->bhqd", p, v)
        return (lambda x, *d: x.transpose(*d))(o, 0, 2, 1, 3).reshape(B, Sq, Hq * Dh) @ wo

    def _B_ref(x, k_cache, v_cache, wq, wo):
        B, Sq, D = x.shape
        H, Dh = 32, 128
        q = (lambda x, *d: x.transpose(*d))((x @ wq).reshape(B, Sq, H, Dh), 0, 2, 1, 3)
        scores = jnp.einsum("bhqd,bhkd->bhqk", q, k_cache) * (Dh ** -0.5)
        p = _softmax(scores, axis=-1)
        o = jnp.einsum("bhqk,bhkd->bhqd", p, v_cache)
        return (lambda x, *d: x.transpose(*d))(o, 0, 2, 1, 3).reshape(B, Sq, H * Dh) @ wo

    a = _A_ref(A_x, A_k_cache, A_v_cache, A_wq, A_wo)
    b = _B_ref(B_x, B_k_cache, B_v_cache, B_wq, B_wo)
    return jnp.concatenate([a, b], axis=-1)
```

```python
import functools
import math
import jax
import jax.numpy as jnp
from jax import lax
import jax.experimental.pallas as pl
import jax.experimental.pallas.tpu as pltpu

M, D, H, DH, SK = 512, 1024, 32, 128, 32
F32, BF, U32 = jnp.float32, jnp.bfloat16, jnp.uint32
C_EXP = (DH ** -0.5) * math.log2(math.e)
ORDER = (1, 3, 2, 4, 0, 5, 6)
SWAP = (False, True, False, False, True, True, True)


def mo(i):
    return i if isinstance(i, int) else pl.multiple_of(i, 16)


def dot(a, b):
    return jnp.dot(a, b, preferred_element_type=F32)


def dot_t(a, b):
    return lax.dot_general(a, b, (((1,), (1,)), ((), ())), preferred_element_type=F32)


def quads(g):
    n = len(g) // 2
    return [[r[c:c + n] for r in g[a:a + n]] for a in (0, n) for c in (0, n)]


def gadd(x, y):
    return [[a + b for a, b in zip(r, s)] for r, s in zip(x, y)]


def gsub(x, y):
    return [[a - b for a, b in zip(r, s)] for r, s in zip(x, y)]


def flip(g):
    n = len(g) // 2
    return [r[n:] + r[:n] for r in g]


def lazy(fn):
    box = []

    def get():
        if not box:
            box.append(fn())
        return box[0]
    return get


def ladd(x, y):
    return [[lazy(lambda a=a, b=b: a() + b()) for a, b in zip(r, s)] for r, s in zip(x, y)]


def lsub(x, y):
    return [[lazy(lambda a=a, b=b: a() - b()) for a, b in zip(r, s)] for r, s in zip(x, y)]


def lhs_terms(g, base=0):
    if len(g) == 1:
        yield base, g[0][0]()
        return
    a11, a12, a21, a22 = quads(g)
    ts = (ladd(a11, a22), ladd(a21, a22), a11, a22, ladd(a11, a12), lsub(a21, a11), lsub(a12, a22))
    for i in (2, 3, 0, 4, 6, 5, 1):
        yield from lhs_terms(ts[i], base + i * 7 ** (len(g).bit_length() - 2))


def rhs_terms(g, base=0):
    if len(g) == 1:
        yield base, g[0][0]()
        return
    b11, b12, b21, b22 = quads(g)
    ts = (ladd(b11, b22), b11, lsub(b12, b22), lsub(b21, b11), b22, ladd(b11, b12), ladd(b21, b22))
    for i in (1, 4, 0, 2, 5, 3, 6):
        yield from rhs_terms(flip(ts[i]) if SWAP[i] else ts[i], base + i * 7 ** (len(g).bit_length() - 2))


def combine(level, prod, base=0, emit=None):
    if level == 0:
        r = prod(base)
        if emit is not None:
            emit(0, 0, r)
        return [[r]]
    n = 2 ** (level - 1)

    def m(i):
        g = combine(level - 1, prod, base + i * 7 ** (level - 1))
        return flip(g) if SWAP[i] else g

    def fin(a, c, g):
        if emit is not None:
            for i in range(n):
                for j in range(n):
                    emit(a * n + i, c * n + j, g[i][j])
        return g
    m2 = m(1)
    m4 = m(3)
    c21 = fin(1, 0, gadd(m2, m4))
    m3 = m(2)
    u = gsub(m3, m2)
    m5 = m(4)
    v = gsub(m4, m5)
    c12 = fin(0, 1, gadd(m3, m5))
    m1 = m(0)
    u = gadd(u, m1)
    v = gadd(v, m1)
    c22 = fin(1, 1, gadd(u, m(5)))
    c11 = fin(0, 0, gadd(v, m(6)))
    return [a + b for a, b in zip(c11, c12)] + [a + b for a, b in zip(c21, c22)]


def order(level, base=0):
    if level == 0:
        return [base]
    return [x for i in ORDER for x in order(level - 1, base + i * 7 ** (level - 1))]


class Side:
    def __init__(self, lag, every):
        self.streams, self.jobs, self.beat, self.seen = [], {}, 0, []
        self.lag, self.every = lag, every

    def add(self, lo, hi, n, gen, fence):
        self.streams.append([int(lo * 8), int(hi * 8), n, gen, 0, fence])

    def at(self, rnd, fn):
        self.jobs.setdefault(rnd, []).append(fn)

    def start_round(self):
        for fn in self.jobs.pop(self.beat // 8, ()):
            fn()

    def result(self, r):
        self.seen += [(r, i) for i in range(0, r.shape[0], 16)]
        return r

    def tick(self):
        pos = len(self.seen) - 16 + self.beat % 8 - self.lag
        self.beat += 1
        for st in self.streams:
            lo, hi, n, gen, done, fence = st
            want = min(n, max(0, -(-n * (self.beat - lo) // (hi - lo))))
            if want > done and pos >= 0 and (self.beat - lo - 1) % self.every == 0:
                r, i = self.seen[pos]
                fence(r[i:i + 8])
            for _ in range(want - done):
                next(gen)
            st[4] = max(want, done)

    def finish(self):
        assert not self.jobs and all(st[4] == st[2] for st in self.streams)


def make(PARTS='pabto', QK=(1, 3, 5, 7), PV=(9, 11, 13, 15), WP=(0, 17), OC=(17, 24.4), XP=(0, 0), WO=(0, 48.5), NODMA=False, FLAGS=None,
         QKA=None, SE=1, LAG=2, EV=2, PZ=True, NOHAZ=False):
    R = 49
    ORD = order(2)
    QKA = QKA or QK

    def kernel(xa, ka, va, wqa, woa, xb, kb, vb, wqb, wob, out,
               x_u, xs_u, ka_u, va_u, kb_u, vb_u, wq_u, wo_u, p_u, t_u, q0_u, q1_u, o_u, part, of0, of1,
               sx, skv, swq, swo, so, zs):
        x_v, xs, ka_v, va_v, kb_v, vb_v, wq_v, wo_v, pp, tt, q0, q1, o_v = [
            r.bitcast(BF) for r in (x_u, xs_u, ka_u, va_u, kb_u, vb_u, wq_u, wo_u, p_u, t_u, q0_u, q1_u, o_u)]
        qb, of = (q0, q1), (of0, of1)
        ppl, ttl = (pltpu.annotate(pp, no_hazard=True), pltpu.annotate(tt, no_hazard=True)) if NOHAZ else (pp, tt)

        class Dummy:
            def start(self): pass
            def wait(self): pass

        def copy(src, dst, sem):
            return Dummy() if NODMA else pltpu.make_async_copy(src, dst, sem)

        def xa_copy():
            return copy(xa, x_v.at[0], sx.at[0])

        def xb_copy(i):
            rs = pl.ds(i * 32, 32)
            return copy(xb.at[:, rs], x_v.at[1, :, rs], sx.at[1 + i])

        def wq_copy(i):
            return copy((wqa, wqb)[i // 8].at[:, pl.ds((i % 8) * 512, 512)], wq_v.at[i], swq.at[i])

        def wq_wait(i):
            copy(wq_v.at[i], wq_v.at[i], swq.at[i]).wait()

        def kva_copy():
            return copy(ka, ka_v, skv.at[0, 0]), copy(va, va_v, skv.at[1, 0])

        def kvb_copy(i):
            hs = pl.ds(i * 8, 8)
            return copy(kb.at[:, hs], kb_v.at[:, hs], skv.at[0, 1 + i]), copy(vb.at[:, hs], vb_v.at[:, hs], skv.at[1, 1 + i])

        def wo_copy(i):
            return copy((woa, wob)[i // 4].at[pl.ds((i % 2) * 2048, 2048), pl.ds((i // 2 % 2) * 512, 512)], wo_v.at[i], swo.at[i])

        def wo_wait(i):
            copy(wo_v.at[i], wo_v.at[i], swo.at[i]).wait()

        @pl.loop(0, 2)
        def _(i):
            zs[i] = 0
        z = zs[0]

        lane = lax.broadcasted_iota(jnp.int32, (16, 128), 1) // SK
        lane_f = lax.broadcasted_iota(jnp.int32, (SK, 128), 1) // SK
        G4 = range(4)
        P0 = 16 * 128

        def prep_x(br, r, n):
            for rr in range(0, n, 16):
                for c in (0, 128):
                    g = [[lazy(lambda i=i, j=j: x_v[br, i, pl.ds(r + rr, 16), pl.ds(j * 256 + c, 128)].astype(F32)) for j in G4] for i in G4]
                    for t, v in lhs_terms(g):
                        xs[pl.ds(mo((br * R + t) * 128 + r + rr), 16), pl.ds(c, 128)] = v.astype(BF)
                        yield

        def prep_wq(i, slot):
            for r in range(0, 256, 16):
                g = [[lazy(lambda a=a, c=c: wq_v[z + i, pl.ds(a * 256 + r, 16), pl.ds(c * 128, 128)].astype(F32)) for c in G4] for a in G4]
                for t, v in rhs_terms(g):
                    if r < 128:
                        pp[pl.ds(P0 + slot * 128 + r, 16), pl.ds(t * 128, 128)] = v.astype(BF)
                    else:
                        tt[pl.ds(1024 + slot * 128 + r - 128, 16), pl.ds(t * 128, 128)] = v.astype(BF)
                    yield

        def prep_wo(i, slot):
            for r in range(0, 512, 16):
                qd, rr = divmod(r, 128)
                g = [[lazy(lambda a=a, c=c: wo_v[z + i, pl.ds(qd * 512 + a * 128 + rr, 16), pl.ds(c * 128, 128)].astype(F32)) for c in G4] for a in G4]
                for t, v in rhs_terms(g):
                    tt[pl.ds(slot * 512 + r, 16), pl.ds(t * 128, 128)] = v.astype(BF)
                    yield

        def fence_wq(w):
            wq_u[16, pl.ds(0, 8), pl.ds(0, 128)] = pltpu.bitcast(w, U32)

        def fence_wo(w):
            wo_u[8, pl.ds(0, 8), pl.ds(0, 128)] = pltpu.bitcast(w, U32)

        def load_round(side, tiles):
            side.start_round()
            if SE > 1 and side.beat // 8 in (24, 49):
                for ref in (p_u, t_u):
                    ref[pl.ds(mo(zs[1] + ref.shape[0] - 8), 8), pl.ds(0, 128)] = jnp.zeros((8, 128), U32)
            got = [[None] * 8 for _ in tiles]
            for j in reversed(range(8)):
                for k, (ref, r, c) in enumerate(tiles):
                    got[k][j] = ref[pl.ds(mo((z if j % SE == 0 else 0) + r + 16 * j), 16), pl.ds(c, 128)]
                side.tick()
            return got

        def attention(side, br, qd, slot, off, qk, pv, oc):
            st, o = {}, [[None] * 4 for _ in G4]

            def scores(bg):
                ps = []
                for j in G4:
                    b = 4 * bg + j
                    qt = jnp.concatenate([qb[slot][pl.ds(mo(z + b * 32), 32), pl.ds(hd * 128, 128)] for hd in G4], axis=0)
                    if br == 0:
                        s = dot_t(pltpu.bitcast(ka_u[b, qd // 2], BF), qt)
                    else:
                        s4 = dot_t(pltpu.bitcast(kb_u[b, pl.ds(qd * 4, 4)].reshape(64, DH), BF), qt)
                        s = s4[:32]
                        for hd in (1, 2, 3):
                            s = jnp.where(lane_f == hd, s4[hd * 32:hd * 32 + 32], s)
                    if j == 0:
                        side.result(s if br == 0 else s4)
                    e = jnp.exp2((s - jnp.max(s, axis=0, keepdims=True)) * C_EXP)
                    l = jnp.sum(e, axis=0, keepdims=True)
                    ps.append(e * pltpu.reciprocal(l, approx=False, full_range=False))
                st[bg] = pltpu.bitcast(jnp.concatenate(ps, axis=0).astype(BF).T, U32)

            def values(bg):
                t = st[bg]
                for hd in G4:
                    th = t[hd * 16:hd * 16 + 16]
                    p = pltpu.bitcast(jnp.concatenate([jnp.where(lane == j, th, jnp.uint32(0)) for j in G4], axis=0), BF)
                    if br == 0:
                        vt = va_u[pl.ds(4 * bg, 4), qd // 2]
                    else:
                        vt = vb_u[pl.ds(4 * bg, 4), qd * 4 + hd]
                    r = dot(p, pltpu.bitcast(vt.reshape(64, DH), BF))
                    of[slot][pl.ds(bg * 128, 128), pl.ds(hd * 128, 128)] = side.result(r) if hd == 0 else r

            def terms():
                for r in range(0, 128, 16):
                    g = [[lazy(lambda i=i, j=j: of[slot][pl.ds(mo(z + i * 128 + r), 16), pl.ds(j * 128, 128)]) for j in G4] for i in G4]
                    for t, v in lhs_terms(g):
                        pp[pl.ds(mo((br * 8 + qd) * 128 + r), 16), pl.ds(t * 128, 128)] = v.astype(BF)
                        yield
            for bg in G4:
                side.at(int(off + qk[bg]), functools.partial(scores, bg))
                side.at(int(off + pv[bg]), functools.partial(values, bg))

            def fence(w):
                of[slot][pl.ds(M, 8), pl.ds(0, 128)] = w
            side.add(off + oc[0], off + oc[1], 8 * R, terms(), fence)

        def qsteps(side, steps):
            seq = [(slot, t) for _, slot in steps for t in ORD]
            w = {}

            def prod(br, slot, t):
                if (slot, t) not in w:
                    i = seq.index((slot, t))
                    pair = seq[i:i + 2]
                    got = load_round(side, [(ref, r0 + s_ * 128, t_ * 128) for s_, t_ in pair for ref, r0 in ((ppl, P0), (ttl, 1024))])
                    for n, key in enumerate(pair):
                        w[key] = jnp.concatenate(got[2 * n] + got[2 * n + 1], axis=0)
                r = dot(xs[pl.ds(mo((br * R + t) * 128), 128), :], w[slot, t])
                return side.result(r) if seq.index((slot, t)) % 2 == 0 else r

            for br, slot in steps:
                def emit(i, j, v):
                    qb[slot][pl.ds(i * 128, 128), pl.ds(j * 128, 128)] = v.astype(BF)
                combine(2, functools.partial(prod, br, slot), emit=emit)
            side.finish()

        def ostep(side, n):
            br = n // 2

            def half(t, hf):
                got = load_round(side, [(ttl, hf * 512 + k * 128, t * 128) for k in G4])
                lhs = jnp.concatenate([pp[pl.ds(mo((br * 8 + hf * 4 + j) * 128), 128), pl.ds(t * 128, 128)] for j in G4], axis=1)
                return side.result(dot(lhs, jnp.concatenate(sum(got, []), axis=0)))
            for t in ORD:
                part[pl.ds(t * 128, 128), :] = half(t, 0)

            def emit(i, j, v):
                o_v[pl.ds(mo(n * M + i * 128), 128), pl.ds(j * 128, 128)] = v.astype(BF)
            combine(2, lambda t: part[pl.ds(mo((z if PZ else 0) + t * 128), 128), :] + half(t, 1), emit=emit)
            side.finish()

        seq = [xa_copy(), wq_copy(0), wq_copy(1), *kva_copy()]
        for i in range(4):
            seq += [xb_copy(i), wq_copy(2 * i + 2), wq_copy(2 * i + 3)]
        for i in range(3):
            seq += [*kvb_copy(i), wq_copy(2 * i + 10), wq_copy(2 * i + 11)]
        seq += [*kvb_copy(3)] + [wo_copy(i) for i in range(8)]
        for c in seq:
            c.start()

        if 'p' in PARTS:
            xa_copy().wait()
            list(prep_x(0, 0, 128))
            wq_wait(0)
            list(prep_wq(0, 0))
            wq_wait(1)
            sd = Side(LAG, EV)
            sd.add(0, 24.9, 16 * R, prep_wq(1, 1), fence_wq)
            qsteps(sd, [(0, 0)])
            for c in kva_copy():
                c.wait()

        def body_q(br, i, _):
            if br == 0:
                xb_copy(i).wait()
            else:
                for c in kvb_copy(i):
                    c.wait()
            n = br * 8 + 2 * i + 2
            wq_wait(n)
            wq_wait(n + 1)
            sd = Side(LAG, EV)
            for k in (0, 1):
                off = 24.5 * k
                sd.add(off + WP[0], off + WP[1], 16 * R, prep_wq(n + k, k), fence_wq)
                attention(sd, br, 2 * i + k, k, off + k, QKA if br == 0 else QK, PV, (OC[0], OC[1] - k))
            if br == 0:
                sd.at(XP[0], lambda: list(prep_x(1, pl.multiple_of(i * 32, 32), 32)))
            qsteps(sd, [(br, 1), (1 if br else (i + 1) // 4, 0)])

        def o_copy(n):
            c0 = n * 512 if isinstance(n, int) else pl.multiple_of(n * 512, 512)
            return pltpu.make_async_copy(o_v.at[pl.ds(mo(n * M), M)], out.at[:, pl.ds(c0, 512)], so)

        def body_o(n, _):
            if not NODMA: o_copy(n - 1).start()
            wo_wait(2 * n + 1)

            @pl.when(n < 3)
            def _():
                wo_wait(2 * n + 2)
            sd = Side(LAG, EV)
            sd.add(WO[0], WO[1], 32 * R, prep_wo(2 * n + 1, 1), fence_wo)
            sd.add(49 + WO[0], 49 + WO[1], 32 * R, prep_wo(jnp.minimum(2 * n + 2, 7), 0), fence_wo)
            ostep(sd, n)

        if 'a' in PARTS:
            lax.fori_loop(0, 4, functools.partial(body_q, 0), None)
        if 'b' in PARTS:
            lax.fori_loop(0, 3, functools.partial(body_q, 1), None)
        if 't' in PARTS:
            for c in kvb_copy(3):
                c.wait()
            wo_wait(0)
            sd = Side(LAG, EV)
            sd.add(0, 20, 32 * R, prep_wo(0, 0), fence_wo)
            attention(sd, 1, 6, 0, 0, QK, PV, (20, 24.9))
            qsteps(sd, [(1, 1)])
            wo_wait(1)
            wo_wait(2)
            sd = Side(LAG, EV)
            sd.add(0, 39, 32 * R, prep_wo(1, 1), fence_wo)
            attention(sd, 1, 7, 1, 0, QK, PV, (39, 48.5))
            sd.add(49 + WO[0], 49 + WO[1], 32 * R, prep_wo(2, 0), fence_wo)
            ostep(sd, 0)
        if 'o' in PARTS:
            lax.fori_loop(1, 4, body_o, None)
        if PARTS == 'pabto' and not NODMA:
            o_copy(3).start()
            pltpu.make_async_copy(out, out, so).wait()
        else:
            for r in (xs, tt, pp, q0, q1, o_v):
                c = pltpu.make_async_copy(r.at[pl.ds(0, 16), pl.ds(0, 256)], out.at[pl.ds(0, 16), pl.ds(0, 256)], so)
                c.start()
                c.wait()

    @jax.jit
    def fn(A_x, A_k_cache, A_v_cache, A_wq, A_wo, B_x, B_k_cache, B_v_cache, B_wq, B_wo):
        any_ = pl.BlockSpec(memory_space=pl.ANY)

        def vm(*shape):
            return pltpu.VMEM((*shape[:-2], shape[-2] // 2, shape[-1]), U32)
        out = pl.pallas_call(
            kernel,
            in_specs=[any_] * 10,
            out_specs=any_,
            out_shape=jax.ShapeDtypeStruct((M, 2 * D), BF),
            scratch_shapes=[
                vm(2, 4, 128, D), vm(2 * R * 128, 256),
                vm(16, 4, SK, DH), vm(16, 4, SK, DH), vm(16, 32, SK, DH), vm(16, 32, SK, DH),
                vm(17, D, 512), vm(9, 2048, 512),
                vm(18 * 128 + 16, R * 128), vm(1024 + 256 + 16, R * 128), vm(M, 512), vm(M, 512),
                vm(4 * M, 512), pltpu.VMEM((R * 128, 128), F32), pltpu.VMEM((M + 8, 512), F32), pltpu.VMEM((M + 8, 512), F32),
                pltpu.SemaphoreType.DMA((5,)), pltpu.SemaphoreType.DMA((2, 5)), pltpu.SemaphoreType.DMA((16,)),
                pltpu.SemaphoreType.DMA((8,)), pltpu.SemaphoreType.DMA(()), pltpu.SMEM((2,), jnp.int32),
            ],
            compiler_params=pltpu.CompilerParams(vmem_limit_bytes=120 * 1024 * 1024, flags=FLAGS),
        )(A_x.reshape(4, 128, D), A_k_cache, A_v_cache, A_wq, A_wo,
          B_x.reshape(4, 128, D), B_k_cache, B_v_cache, B_wq, B_wo)
        return out.reshape(16, 32, 2 * D)

    return fn


pallas_concat_heads__gqa_block_cached__mha_block_cached__near_ridge_kernel = make(LAG=2, EV=4, SE=4)
```

```python
import functools
import math

import jax
import jax.numpy as jnp
from jax import lax
import jax.experimental.pallas as pl
import jax.experimental.pallas.tpu as pltpu

M, D, DH, SK = 512, 1024, 128, 32
R = 49
G4 = range(4)
F32, BF16, U32 = jnp.float32, jnp.bfloat16, jnp.uint32
EXP_SCALE = DH ** -0.5 * math.log2(math.e)

RUN = (1, 3, 2, 4, 0, 5, 6)
ORDER = [7 * i + j for i in RUN for j in RUN]
SWAPPED = (False, True, False, False, True, True, True)


def _once(fn):
    box = []

    def get():
        if not box:
            box.append(fn())
        return box[0]

    return get


def _operands(g, left, base=0):
    if len(g) == 1:
        yield base, g[0][0]()
        return
    n = len(g) // 2
    g11, g12, g21, g22 = ([r[c:c + n] for r in g[a:a + n]] for a in (0, n) for c in (0, n))

    def both(op, x, y):
        return [[_once(lambda a=a, b=b: op(a(), b())) for a, b in zip(r, s)] for r, s in zip(x, y)]

    add, sub = functools.partial(both, lax.add), functools.partial(both, lax.sub)
    if left:
        sums = (add(g11, g22), add(g21, g22), g11, g22, add(g11, g12), sub(g21, g11), sub(g12, g22))
    else:
        sums = (add(g11, g22), g11, sub(g12, g22), sub(g21, g11), g22, add(g11, g12), add(g21, g22))
    for i in (2, 3, 0, 4, 6, 5, 1) if left else (1, 4, 0, 2, 5, 3, 6):
        s = [r[::-1] for r in sums[i]] if SWAPPED[i] and not left else sums[i]
        yield from _operands(s, left, base + i * (7 if n == 2 else 1))


def _recombine(emit, early):
    add, sub = lax.add, lax.sub
    m2 = yield
    m4 = yield
    emit(1, 0, add(m2, m4))
    m3 = yield
    m5 = yield
    emit(0, 1, add(m3, m5))
    m1 = yield
    m6 = yield
    if early == 2:
        emit(1, 1, add(add(sub(m3, m2), m1), m6))
    elif early == 1:
        emit(1, 1, add(add(sub(m1, m2), m3), m6))
    else:
        emit(1, 1, add(sub(add(m6, m1), m2), m3))
    m7 = yield
    if early == 2:
        emit(0, 0, add(add(sub(m4, m5), m1), m7))
    elif early == 1:
        emit(0, 0, add(add(m7, m1), sub(m4, m5)))
    else:
        emit(0, 0, add(sub(add(m7, m1), m5), m4))
    yield


def _strassen(product, emit, early):
    outer = {}
    for a in (0, 1):
        for c in (0, 1):
            outer[a, c] = _recombine(lambda i, j, v, a=a, c=c: emit(2 * i + a, 2 * j + c, v), early[1])
            next(outer[a, c])
    for i in RUN:
        inner = _recombine(lambda a, c, v, i=i: outer[a, c ^ SWAPPED[i]].send(v), early[0])
        next(inner)
        for j in RUN:
            inner.send(product(7 * i + j))


def _recombine_cost(i, cf):
    o, p = divmod(i % R, 7)
    stores = ((1, 1, 1, 1, 1, 0, 0), (1, 1, 1, 1, 2, 0, 0), (1, 1, 2, 1, 2, 0, 0))
    adds = ((0, 1, 0, 1, 0, 3, 3), (0, 1, 0, 2, 2, 1, 2), (0, 1, 1, 2, 2, 1, 1))
    e0, e1 = cf["early"]
    st, al = 16 * stores[e0][p], 16 * adds[e0][p]
    if p in (1, 3, 5, 6):
        st += 16 * stores[e1][o] + 8 * (o in (1, 3, 5, 6))
        al += 16 * adds[e1][o] + 8 * (o in (1, 3, 5, 6))
    return (st + cf["alu"] * al) / cf["cap"]


class _Source:
    def __init__(self, view, spare):
        self.view, self.spare, self.due, self.last = view, spare, None, -99

    def block(self, row, j):
        if self.due:
            self.last, res, i = self.due
            w = lax.slice_in_dim(res, i, i + 8)
            w = lax.convert_element_type(w, self.spare.dtype)
            self.spare[pl.ds(0, w.shape[0]), pl.ds(0, 128)] = w
            self.due = None
        if len(self.view.shape) == 3:
            return self.view[j // 2, pl.ds(row, 16), pl.ds(j % 2 * 128, 128)]
        return self.view[pl.ds(row, 16), pl.ds(j * 128, 128)]


class _Schedule:
    def __init__(self, cf):
        self.cf, self.streams, self.jobs, self.seen = cf, [], {}, []
        self.round, self.beat, self.time, self.short = 0, 0, 0.0, 0

    def spread(self, lo, hi, work):
        scale = (hi - lo) / sum(w["steps"] * w["cost"] for w in work)
        for w in work:
            self.streams.append(dict(w, lo=lo, hi=lo + w["steps"] * w["cost"] * scale, done=0))
            lo = self.streams[-1]["hi"]

    def at(self, rnd, fn):
        self.jobs.setdefault(rnd, []).append(fn)

    def start_round(self):
        for s in self.streams:
            if s.get("wait") and self.time >= s["lo"] - 0.3:
                s.pop("wait")()
                s["lo"] = self.time
        for fn in self.jobs.pop(self.round, ()):
            fn()
        self.round += 1

    def result(self, res, room):
        self.seen += [(res, i, room) for i in range(0, res.shape[0], 16)]
        return res

    def tick(self, beats):
        for beat in [*range(-self.short, 0), *beats]:
            pos = len(self.seen) - 16 + beat
            self.time += (self.seen[pos][2] if pos >= 0 else self.cf["head"] * bool(self.seen)) / 8
            self.beat += 1
            pos -= self.cf["lag"]
            for s in self.streams:
                due = math.ceil(s["steps"] * (self.time - s["lo"]) / (s["hi"] - s["lo"]))
                due = 0 if s.get("wait") else min(s["steps"], due)
                if due > s["done"] and pos >= 0 and self.beat >= s["src"].last + self.cf["every"]:
                    s["src"].due = (self.beat, *self.seen[pos][:2])
                while s["done"] < due:
                    next(s["gen"])
                    s["done"] += 1
        self.short = 0

    def weights(self, tiles):
        self.start_round()
        n = self.cf["rows2"] if self.short or not self.seen else self.cf["rows"]
        got = [[] for _ in tiles]
        for j in range(8 - n, -1, -n):
            for rows, (ref, t) in zip(got, tiles):
                rows.insert(0, ref[pl.ds(16 * j, 16 * n), pl.ds(t * 128, 128)])
            self.tick(range(8 - n - j, 8 - j))
        return got

    def finish(self):
        self.start_round()
        self.tick(range(16))
        assert not self.jobs and all(s["done"] == s["steps"] for s in self.streams)


_DEFAULT = dict(qk=(), pv=(), qk2=(), pv2=(), lag=1, every=2, rows=2, rows2=4, head=0.8, tail=0.3, gap=0.5,
                room_qk=0.5, room_pv=0.4, softmax=0.3, alu=0.25, cap=130, o_cost=0.9, early=(2, 1),
                keep_w=15, keep_o=15, adj=(0,) * R)
_TUNED = dict(
    p=dict(every=3, head=0.7, tail=0.75, keep_w=11),
    s=dict(qk=(2, 3, 5, 7), pv=(7, 10, 24, 25), lag=2, rows=8, rows2=2, head=0.89, tail=0.25, gap=6.85, room_qk=0.69,
           room_pv=0.28, softmax=0.53, cap=128, o_cost=1.27, early=(1, 0), keep_w=9, keep_o=11, adj=(0.08, 0.14,
           -0.08, 0.03, 0.12, -0.19, 0.04, 0.03, 0.07, -0.16, -0.07, 0.01, 0.02, 0.02, 0.01, 0.06, 0.01, -0.01, 0.02,
           0.06, 0.0, 0.02, 0.0, 0.0, 0.01)),
    a=dict(qk=(3, 3, 4, 5), pv=(16, 16, 23, 25), lag=2, rows2=1, head=0.86, tail=0.38, softmax=0.56, alu=0.14,
           o_cost=0.99, early=(1, 0), keep_o=1, adj=(-0.09, -0.01, 0.01, 0.38, -0.1, -0.02, -0.07, 0, 0.0, 0, 0.2,
           0.0, -0.09, 0.04, 0.02, 0.04, 0.12, 0.05, 0.0, 0.01, 0.11, -0.11, 0, -0.13, 0)),
    c=dict(qk=(3, 3, 4, 4), pv=(11, 18, 18, 18), qk2=(27, 28, 29, 30), pv2=(40, 41, 48, 49), every=1, rows2=8,
           head=0.28, tail=0.25, room_pv=0.37, softmax=0.5, alu=0.07, o_cost=0.8, keep_o=9, adj=(0.01, -0.17, -0.13,
           0.09, -0.1, -0.11, -0.35, -0.22, -0.06, 0.01, 0.01, 0.22, -0.16, 0.03, 0.03, 0.27, -0.12, 0.16, -0.03,
           -0.05, -0.1, -0.03, 0.05, 0.06, -0.04, 0.05, -0.6, -0.55, -0.6, 0.27, -0.11, -0.23, -0.0, 0.15, -0.09,
           -0.12, 0.01, -0.11, -0.25, 0.06, 0.12, 0.04, -0.13, -0.04, 0.26, -0.3, -0.49, -0.02, 0.03)),
    b=dict(qk=(2, 3, 5, 6), pv=(13, 16, 18, 19), qk2=(27, 28, 29, 30), pv2=(42, 42, 46, 49), rows2=1, head=0.59,
           tail=0.12, gap=0.42, room_qk=0.71, softmax=0.22, alu=0.36, o_cost=0.83, adj=(-0.03, -0.11, 0.03, -0.1,
           -0.08, -0.13, 0, -0.0, 0, 0, 0.06, 0, 0.03, -0.2, 0.03, 0.01, 0.05, 0, 0.07, 0.02, 0, 0, 0, 0, 0, 0, -0.2,
           0.0, 0, 0, 0.1, 0, 0, 0, 0, 0, 0, 0, 0, 0.2, 0, 0, 0, 0, 0.1, 0, 0, 0, 0.1)),
    t=dict(qk=(1, 2, 4, 4), pv=(16, 18, 20, 22), lag=0, every=1, rows=4, rows2=8, tail=1.32, room_pv=0.67,
           softmax=0.32, alu=0.24, cap=132, o_cost=1.06, early=(1, 0), keep_w=9, keep_o=9, adj=(0.3, 0.03, 0.23,
           -0.07, 0.12, 0.1, 0.12, 0.19, -0.14, 0.29, 0.03, 0.09, 0.04, 0.38, 0.06, -0.39, 0.1, 0.13, -0.1, 0.07,
           0.24, -0.43, 0.2, 0.07, 0.1)),
    u=dict(qk=(4, 4, 8, 8), pv=(18, 22, 22, 28), lag=4, rows2=1, head=0.84, gap=0.31, room_qk=0.51, room_pv=0.6,
           softmax=0.28, cap=229, early=(2, 2), keep_o=11, adj=(-0.03, -0.28, -0.07, -0.43, -0.19, -0.19, -0.17, 0.07,
           0.01, -0.1, 0.03, -0.04, -0.01, 0.01, 0.12, 0.07, 0.09, 0.07, -0.01, -0.29, 0.15, -0.01, 0.1, 0.08, 0.09,
           0.03, 0.12, 0.08, -0.0, 0.03, -0.16, 0.03, 0.02, 0.08, 0.07, 0.1, 0.04, 0.05, 0.12, 0.03, 0.04, 0.11, 0.18,
           0.06, 0.11, 0.01, 0.02, 0, 0)),
    o=dict(lag=3, every=3, head=0.97, tail=0.32, gap=0.42, cap=300, early=(2, 2), keep_o=13, adj=(0.02, 0.01, 0.01,
           0.02, 0.02, 0, 0, 0.01, 0, 0.02, 0, -0.08, 0.01, 0.02, 0.01, 0.01, 0, 0, 0.01, 0, 0.02, 0.02, 0.01, 0.01,
           0, 0.02, 0.02, 0.01, 0, 0.01, 0, 0.02, 0.02, 0.02, 0.01, 0.03, 0, 0.01, 0.04, 0, 0.01, 0, 0.02, 0, 0.01,
           0.01, 0.01, 0.01, -0.1)),
)


def _dot(a, b):
    return lax.dot_general(a, b, (((1,), (0,)), ((), ())), preferred_element_type=F32)


def _dot_t(a, b):
    return lax.dot_general(a, b, (((1,), (1,)), ((), ())), preferred_element_type=F32)


def _bf16(v):
    return lax.convert_element_type(v, BF16)


def _tile(i, n=1):
    return pl.ds(i * 128 if isinstance(i, int) else pl.multiple_of(i * 128, 128), n * 128)


def _kernel(xa, ka, va, wqa, woa, xb, kb, vb, wqb, wob, out,
            x_v, xs_w, kva, kvb, wq_v, wo_v, os_w, ws_w, q_w, out_v, partial, o_f32, sems, zeros):
    xs, os_, ws, q_v = (r.bitcast(BF16) for r in (xs_w, os_w, ws_w, q_w))
    cfg = {k: dict(_DEFAULT, **v) for k, v in _TUNED.items()}

    def x_copy(c):
        return (xa, xb)[c // 4].at[:, _tile(c % 4 * 2, 2)], x_v.at[c]

    def wq_copy(quad, k=0, n=8):
        return (wqa, wqb)[quad // 8].at[_tile(k, n), _tile(quad % 8 * 4, 4)], wq_v.at[quad, _tile(k, n)]

    def wo_copy(i):
        return (wob, woa)[i // 4].at[_tile(i % 2 * 16, 16), _tile(i // 2 % 2 * 4, 4)], wo_v.at[i]

    def kv_copy(k, v, dst, h, n):
        hs = pl.ds(h, n)
        return [(k.at[:, hs], dst.at[0, :, hs]), (v.at[:, hs], dst.at[1, :, hs])]

    groups = [[x_copy(c), wq_copy(0, 2 * c, 2)] for c in G4]
    groups += [[wq_copy(1, 0, 4)], [wq_copy(1, 4, 4)]]
    groups += [kv_copy(ka, va, kva, g, 1) for g in (0, 1)]
    groups += [[wq_copy(n)] for n in range(2, 6)]
    groups += [[wq_copy(6 + 2 * i), wq_copy(7 + 2 * i), *kv_copy(ka, va, kva, 2 + i, 1),
                x_copy(4 + 2 * i), x_copy(5 + 2 * i)] for i in range(2)]
    groups += [[wq_copy(10 + 2 * i), wq_copy(11 + 2 * i), *kv_copy(kb, vb, kvb, 8 * i, 8)]
               for i in range(3)]
    groups += [[wo_copy(0), *kv_copy(kb, vb, kvb, 24, 8)], [wo_copy(1), wo_copy(2)]]
    groups += [[wo_copy(i)] for i in range(3, 8)]
    out_sem = sems.at[len(groups)]
    for g in [*range(7), 8, 9, 10, 7, *range(11, 24)]:
        for src, dst in groups[g]:
            pltpu.make_async_copy(src, dst, sems.at[g]).start()

    def wait(g):
        for src, dst in groups[g]:
            pltpu.make_async_copy(src, dst, sems.at[g]).wait()

    def wait_one(i, choices):
        for k, gs in enumerate(choices):
            @pl.when(i == k)
            def _():
                for g in gs:
                    wait(g)

    @pl.loop(0, 2)
    def _(i):
        zeros[i] = 0

    z, y = zeros[0], zeros[1]

    def sums(left, src, dsts, keep, cost=1.0, first=0):
        def gen():
            for c, dst in enumerate(dsts):
                for r in range(0, 128, 16):
                    held = {}

                    def get(i, j):
                        if (i, j) not in held:
                            held[i, j] = lax.convert_element_type(src.block(c * 512 + i * 128 + r, j), F32)
                        return held[i, j]

                    grid = [[functools.partial(get, i, j) for j in G4] for i in G4]
                    for n, (t, v) in enumerate(_operands(grid, left)):
                        if n % 7 == 6:
                            for i, j in list(held):
                                if not keep >> (i // 2 * 2 + j // 2) & 1:
                                    del held[i, j]
                        dst[pl.ds(first + r, 16), _tile(t)] = _bf16(v)
                        yield

        return dict(steps=8 * R * len(dsts), cost=cost, gen=gen(), src=src)

    def x_sums(cf, i):
        return sums(True, _Source(x_v.at[pl.ds(y + 2 * i, 2)], x_v.at[8]), [xs.at[i]], cf["keep_w"])

    def wq_sums(cf, quad, slot):
        dsts = [os_.at[_tile(16 + slot)], ws.at[8 + slot]]
        return sums(False, _Source(wq_v.at[y + quad], wq_v.at[16]), dsts, cf["keep_w"])

    def wo_sums(cf, i, half):
        dsts = [ws.at[half * 4 + c] for c in G4]
        return sums(False, _Source(wo_v.at[y + i], wo_v.at[8]), dsts, cf["keep_w"])

    def o_sums(cf, slot, quad, view=None):
        dst, first = (os_.at[_tile(quad)], 0) if view is None else (view, quad * 128)
        return sums(True, _Source(o_f32.at[y + slot], o_f32.at[4]), [dst], cf["keep_o"], cf["o_cost"], first)

    def attention(sch, gqa, quad, q_slot, o_slot, qk, pv):
        q, st = q_v.at[y + q_slot], {}

        def scores(bg):
            if gqa:
                sch.short += 2
            else:
                sch.tick(range(8))
            if bg == 0:
                st["q"] = [lax.concatenate([q[pl.ds(b * 32, 32), _tile(h)] for h in G4], 0) for b in range(16)]
            probs = []
            for b in range(4 * bg, 4 * bg + 4):
                if gqa:
                    s = raw = _dot_t(kva[0, b, quad // 2], st["q"][b])
                else:
                    raw = _dot_t(kvb[0, b, pl.ds(quad * 4, 4)].reshape(4 * SK, DH), st["q"][b])
                    head = lax.broadcasted_iota(jnp.int32, (SK, 128), 1) // 32
                    s = raw[:SK]
                    for h in (1, 2, 3):
                        s = lax.select(head == h, raw[h * SK:(h + 1) * SK], s)
                if b % 4 == 0:
                    sch.result(raw, sch.cf["room_qk"])
                e = jnp.exp2((s - jnp.max(s, axis=0, keepdims=True)) * EXP_SCALE)
                total = jnp.sum(e, axis=0, keepdims=True)
                probs.append(e * pltpu.reciprocal(total, approx=False, full_range=False))
            st[bg] = pltpu.bitcast(_bf16(lax.concatenate(probs, 0)).T, U32)

        def values(bg):
            sch.tick(range(8))
            batch = lax.broadcasted_iota(jnp.int32, (16, 128), 1) // SK
            for h in G4:
                p = st[bg][h * 16:(h + 1) * 16]
                p = lax.concatenate([lax.select(batch == j, p, jnp.zeros_like(p)) for j in G4], 0)
                v = kva[1, pl.ds(4 * bg, 4), quad // 2] if gqa else kvb[1, pl.ds(4 * bg, 4), quad * 4 + h]
                o = _dot(pltpu.bitcast(p, BF16), v.reshape(4 * SK, DH))
                o_f32[o_slot, _tile(bg), _tile(h)] = o if h else sch.result(o, sch.cf["room_pv"])

        for bg in G4:
            sch.at(qk[bg], functools.partial(scores, bg))
            sch.at(pv[bg], functools.partial(values, bg))
        return (1 if gqa else 4) * sch.cf["room_qk"] + 4 * sch.cf["room_pv"]

    def project_q(cf, gqa, steps, begin=0):
        sch, n = _Schedule(cf), len(steps) * R
        rounds = [[0]] * (n % 2) + [[i, i + 1] for i in range(n % 2, n, 2)]
        room = [max(0.1, 1 + d - sum(_recombine_cost(i, cf) for i in r) * 2 / len(r)) for r, d in zip(rounds, cf["adj"])]
        for r in cf["qk"] + cf["qk2"]:
            room[r] = max(0.05, room[r] - cf["softmax"])
        att = [attention(sch, gqa, quad, 1 - slot, o_slot, cf["qk" + k], cf["pv" + k])
               for k, (_, slot, quad, o_slot, _) in zip(("", "2"), steps)]
        end = (1 + n % 2 / 2) * cf["head"] + sum(room) - n % 2 * room[0] / 2 + sum(att) - cf["tail"]
        cuts = [begin, end] if n % 2 else [begin, cf["head"] + sum(room[:22]) + att[0] - cf["gap"], end]
        for k, step in enumerate(steps):
            sch.spread(cuts[k], cuts[k + 1], step[4])
        rhs = [(os_.at[_tile(z + 16 + step[1])], ws.at[z + 8 + step[1]]) for step in steps]
        opens, w = {r[0]: (r, rm) for r, rm in zip(rounds, room)}, {}

        def product(k, lhs, t):
            def rows(r, m):
                return lax.concatenate([ref[pl.ds(r, m), _tile(t)] for ref in lhs], 1)

            i = k * R + ORDER.index(t)
            if i not in opens:
                return _dot(rows(0, 128), w[i])
            members, rm = opens[i]
            got = sch.weights([(ref, ORDER[j % R]) for j in members for ref in rhs[j // R]])
            for m, j in enumerate(members):
                w[j] = lax.concatenate(got[2 * m] + got[2 * m + 1], 0)
            if len(members) == 2:
                return sch.result(_dot(rows(0, 128), w[i]), rm)
            return lax.concatenate([sch.result(_dot(rows(0, 64), w[i]), rm), _dot(rows(64, 64), w[i])], 0)

        for k, (block, slot, *_) in enumerate(steps):
            def emit(i, j, v, dst=q_v.at[slot]):
                dst[_tile(i), _tile(j)] = _bf16(v)

            _strassen(functools.partial(product, k, (xs.at[2 * block], xs.at[2 * block + 1])), emit, cf["early"])
        sch.finish()

    last = ((0, 1), (1, 0))

    def send(n, i, j):
        src, dst = out_v.at[n * 4 + j, _tile(i)], out.at[_tile(i), _tile((n + 2) % 4 * 4 + j)]
        pltpu.make_async_copy(src, dst, out_sem).start()

    def project_o(sch, n, att, views, first, work):
        cf = sch.cf
        room = [max(0.1, 1 + cf["adj"][i] - _recombine_cost(i, cf)) for i in range(R)]
        mid = R - 2 + cf["head"] + att
        sch.spread(0, mid - cf["gap"], work[0])
        sch.spread(mid, mid + 2 + sum(room) - cf["tail"], work[1])
        rhs = ws.at[pl.ds(z, 8)]

        def product(t, half):
            got = sch.weights([(rhs.at[half * 4 + k], t) for k in G4])
            a = [views[half][_tile(first + half * 4 + k), _tile(t)] for k in G4]
            if views[0] is not views[1]:
                a[0] = lax.concatenate([views[1 - half][pl.ds((first + half * 4) * 128, 16), _tile(t)], a[0][16:]], 0)
            res = _dot(lax.concatenate(a, 1), lax.concatenate(sum(got, []), 0))
            return sch.result(res, room[ORDER.index(t)] if half else 1.0)

        for t in ORDER:
            partial[_tile(t), :] = product(t, 0)
        done = partial.at[_tile(z, R)]

        def emit(i, j, v):
            out_v.at[n * 4 + j][_tile(i), :] = _bf16(v)
            if (i, j) not in last:
                sch.at(sch.round + 2, functools.partial(send, n, i, j))

        _strassen(lambda t: lax.add(done[_tile(t), :], product(t, 1)), emit, cf["early"])
        sch.finish()

    def first_quad(c0, i, _):
        wait_one(i, ([c0], [c0 + 1]))
        c, sch = c0 + i, _Schedule(cfg["p"])
        if c0:
            sch.spread(0, 8 + sch.cf["head"] - sch.cf["tail"], [x_sums(sch.cf, i)])
        for r in G4:
            for j in (0, 2):
                sch.tick(range(8))
                res = _dot(x_v[c, _tile(r), :], wq_v[0, _tile(2 * c, 2), _tile(j, 2)])
                sch.result(res[:, :128], 1.0)
                for k in (0, 1):
                    v = res[:, k * 128:(k + 1) * 128] + partial[_tile(r * 4 + j + k), :]
                    partial[_tile(r * 4 + j + k), :] = v
                    if c0:
                        q_v.at[0][_tile(r), _tile(j + k)] = _bf16(v)
        sch.finish()

    def part_p():
        partial[_tile(0, 16), :] = jnp.zeros((16 * 128, 128), F32)
        for c0 in (0, 2):
            lax.fori_loop(0, 2, functools.partial(first_quad, c0), None)
        gen = wq_sums(cfg["p"], 1, 1)["gen"]
        for g in (4, 5):
            wait(g)
            for _ in range(8 * R):
                next(gen)

    def part_s():
        cf = cfg["s"]
        wait(6)
        project_q(cf, True, [(0, 1, 0, 0, [dict(wq_sums(cf, 2, 0), wait=functools.partial(wait, 8))])], cf["gap"])

    def body_a(i, _):
        n, cf = i + 2, cfg["a"]
        wait_one(i, ([9], [10, 7], [11]))
        project_q(cf, True, [(0, n % 2, n - 1, i // 2 * 2, [o_sums(cf, 0, n - 2), wq_sums(cf, n + 1, (n + 1) % 2)])])

    def body_c(i, _):
        n, cf = 5 + 2 * i, cfg["c"]
        wait_one(i, ([12], [13]))
        project_q(cf, True, [(0, 1, n - 1, 0, [x_sums(cf, 2 + i), wq_sums(cf, n + 1, 0)]),
                             (i, 0, n, 3 - 3 * i, [o_sums(cf, 0, n - 1), wq_sums(cf, n + 2, 1)])])

    def body_b(i, _):
        n, cf = 9 + 2 * i, cfg["b"]
        wait_one(i, ([14], [15], [16]))
        project_q(cf, False, [(1, 1, n - 9, 0, [o_sums(cf, 0, n - 2), wq_sums(cf, n + 1, 0)]),
                              (1, 0, n - 8, 0, [o_sums(cf, 0, n - 1), wq_sums(cf, n + 2, 1)])])

    def part_t():
        wait(17)
        project_q(cfg["t"], False, [(1, 1, 6, 1, [wo_sums(cfg["t"], 0, 0)])])

    def part_u():
        cf = cfg["u"]
        sch = _Schedule(cf)
        att = attention(sch, False, 7, 1, 0, cf["qk"], cf["pv"])
        v0, v1 = os_.at[_tile(y, 16)], os_.at[_tile(z, 16)]
        work0 = [o_sums(cf, 0, 13, v0), o_sums(cf, 1, 14, v0),
                 dict(wo_sums(cf, 1, 1), wait=functools.partial(wait, 18)),
                 o_sums(cf, 2, 3, v0), o_sums(cf, 0, 15, v0)]
        work1 = [o_sums(cf, 3, 5, v1), wo_sums(cf, 2, 0)]
        project_o(sch, 0, att, (v0, v1), 8, (work0, work1))

    def body_o(i, _):
        n, cf = i + 1, cfg["o"]
        wait_one(i, ([19, 20], [21, 22], [23]))
        sch = _Schedule(cf)
        for k, ij in enumerate(last):
            sch.at(2 + k, functools.partial(send, i, *ij))
        work = [wo_sums(cf, 2 * n + 1, 1)], [wo_sums(cf, jnp.minimum(2 * n + 2, 7), 0)]
        project_o(sch, n, 0, [os_.at[_tile(8 - n // 2 * 8, 8)]] * 2, 0, work)

    def first_phase():
        part_p()
        part_s()
        lax.fori_loop(0, 3, body_a, None)
        lax.fori_loop(0, 2, body_c, None)
        lax.fori_loop(0, 3, body_b, None)

    def second_phase():
        part_t()
        part_u()
        lax.fori_loop(0, 3, body_o, None)

    @pl.loop(0, 2)
    def _(phase):
        lax.cond(phase == 0, first_phase, second_phase)

    for ij in last:
        send(3, *ij)
    pltpu.make_async_copy(out, out, out_sem).wait()


@jax.jit
def pallas_concat_heads__gqa_block_cached__mha_block_cached__near_ridge_kernel(
    A_x: jax.Array,
    A_k_cache: jax.Array,
    A_v_cache: jax.Array,
    A_wq: jax.Array,
    A_wo: jax.Array,
    B_x: jax.Array,
    B_k_cache: jax.Array,
    B_v_cache: jax.Array,
    B_wq: jax.Array,
    B_wo: jax.Array,
):
    def words(*shape):
        return pltpu.VMEM((*shape[:-2], shape[-2] // 2, shape[-1]), U32)

    hbm = pl.BlockSpec(memory_space=pl.ANY)
    out = pl.pallas_call(
        _kernel,
        in_specs=[hbm] * 10,
        out_specs=hbm,
        out_shape=jax.ShapeDtypeStruct((M, 2 * D), BF16),
        scratch_shapes=[
            pltpu.VMEM((9, M, 256), BF16),
            words(4, 128, R * 128),
            pltpu.VMEM((2, 16, 4, SK, DH), BF16),
            pltpu.VMEM((2, 16, 32, SK, DH), BF16),
            pltpu.VMEM((17, D, 512), BF16),
            pltpu.VMEM((9, 2048, 512), BF16),
            words(18 * 128, R * 128),
            words(10, 128, R * 128),
            words(2, M, 512),
            pltpu.VMEM((16, M, 128), BF16),
            pltpu.VMEM((R * 128, 128), F32),
            pltpu.VMEM((5, M, 512), F32),
            pltpu.SemaphoreType.DMA((25,)),
            pltpu.SMEM((2,), jnp.int32),
        ],
        compiler_params=pltpu.CompilerParams(
            vmem_limit_bytes=120 * 1024 * 1024, disable_bounds_checks=True, disable_semaphore_checks=True),
    )(A_x.reshape(M, D), A_k_cache, A_v_cache, A_wq, A_wo, B_x.reshape(M, D), B_k_cache, B_v_cache, B_wq, B_wo)
    return out.reshape(*A_x.shape[:2], 2 * D)
```
